```python
import os as _os
_os.environ.setdefault("JAX_PLATFORMS", "cpu")
import jax
import jax.numpy as jnp

def _softmax(x, axis=-1):
    return jax.nn.softmax(x, axis=axis)
def _gelu(x):
    return jax.nn.gelu(x, approximate=True)
def _silu(x):
    return jax.nn.silu(x)
def _sigmoid(x):
    return jax.nn.sigmoid(x)
def _layernorm(x, axis=-1, eps=1e-5):
    m = jnp.mean(x, axis=axis, keepdims=True)
    v = jnp.var(x, axis=axis, keepdims=True)
    return (x - m) / jnp.sqrt(v + eps)
def _scatter_add(tgt, idx, src, axis=0):
    return tgt.at[idx].add(src)
def _segment_sum(src, seg, n):
    return jax.ops.segment_sum(src, seg, n)
class _Rng:
    def __init__(self, key):
        self._k = key
    def _next(self):
        self._k, sub = jax.random.split(self._k)
        return sub
    def normal(self, shape):
        return jax.random.normal(self._next(), shape, dtype=jnp.bfloat16)
    def randint(self, lo, hi, shape):
        return jax.random.randint(self._next(), shape, lo, hi, dtype=jnp.int32)
    def uniform(self, shape, lo=0.0, hi=1.0):
        return jax.random.uniform(self._next(), shape, jnp.bfloat16, lo, hi)
    def permutation(self, n):
        return jax.random.permutation(self._next(), n)


kernel_name = 'concat_heads__sliding_local_dilated__linear_attn_block__prompt'

def setup_inputs():
    _rng = _Rng(jax.random.key(int.from_bytes(__import__("os").urandom(4), "little")))
    _w = (lambda a: (lambda t: t.astype(jnp.bfloat16) if jnp.issubdtype(t.dtype, jnp.floating) else t)(jnp.asarray(a)))
    def _A_setup():
        B, S, D = 1, 2048, 640
        return {
            "x": _w((lambda *s: _rng.normal(s) * 0.2)(B, S, D)),
            "wqkv": _w((lambda *s: _rng.normal(s) * 0.2)(D, 3 * D)),
            "wo": _w((lambda *s: _rng.normal(s) * 0.05)(D, D)),
        }
    _A_in = _A_setup()

    def _B_setup():
        B, S, D = 1, 2048, 640
        return {
            "x": _w((lambda *s: _rng.normal(s) * 0.05)(B, S, D)),
            "wqkv": _w((lambda *s: _rng.normal(s) * 1.6)(D, 3 * D)),
            "wo": _w((lambda *s: _rng.normal(s) * 0.4)(D, D)),
        }
    _B_in = _B_setup()

    return {
        "A_x": _A_in["x"],
        "A_wqkv": _A_in["wqkv"],
        "A_wo": _A_in["wo"],
        "B_x": _B_in["x"],
        "B_wqkv": _B_in["wqkv"],
        "B_wo": _B_in["wo"],
    }

def reference(A_x, A_wqkv, A_wo, B_x, B_wqkv, B_wo):
    def _A_ref(x, wqkv, wo):
        B, S, D = x.shape
        H = 32; Dh = D // H
        W, dil = 8, 2
        qkv = (lambda x, *d: x.transpose(*d))((x @ wqkv).reshape(B, S, 3, H, Dh), 2, 0, 3, 1, 4)
        q, k, v = qkv[0], qkv[1], qkv[2]
        scale = Dh ** -0.5
        pos = jnp.arange(S)
        off = jnp.arange(W) * dil
        idx = pos[:, None] - off[None, :]
        mask = idx >= 0
        idx_c = jnp.where(mask, idx, 0).reshape(-1)
        kg = k[:, :, idx_c, :].reshape(B, H, S, W, Dh)
        vg = v[:, :, idx_c, :].reshape(B, H, S, W, Dh)
        logits = jnp.einsum("bhsd,bhswd->bhsw", q, kg) * scale
        logits = jnp.where(mask[None, None, :, :], logits, -1e9)
        attn = _softmax(logits, axis=-1)
        o = jnp.einsum("bhsw,bhswd->bhsd", attn, vg)
        return (lambda x, *d: x.transpose(*d))(o, 0, 2, 1, 3).reshape(B, S, D) @ wo

    def _B_ref(x, wqkv, wo):
        B, S, D = x.shape
        H = 32; Dh = D // H
        qkv = (lambda x, *d: x.transpose(*d))((x @ wqkv).reshape(B, S, 3, H, Dh), 2, 0, 3, 1, 4)
        q, k, v = qkv[0], qkv[1], qkv[2]
        phi = lambda t: jnp.where(t > 0, t + 1, jnp.exp(t)) + 1e-6
        pq, pk = phi(q), phi(k)
        kv = jnp.einsum("bhsd,bhse->bhde", pk, v)
        z = jnp.einsum("bhsd->bhd", pk)
        num = jnp.einsum("bhqd,bhde->bhqe", pq, kv)
        den = jnp.einsum("bhqd,bhd->bhq", pq, z)[..., None] + 1e-6
        o = num / den
        return (lambda x, *d: x.transpose(*d))(o, 0, 2, 1, 3).reshape(B, S, D) @ wo

    a = _A_ref(A_x, A_wqkv, A_wo)
    b = _B_ref(B_x, B_wqkv, B_wo)
    return jnp.concatenate([a, b], axis=-1)
```

```python
import contextlib
import functools
import os

import jax
import jax.numpy as jnp
from jax import lax
import jax.experimental.pallas as pl
import jax.experimental.pallas.tpu as pltpu

S, D, H, DH, W, DIL = 2048, 640, 32, 20, 8, 2
NT_ = D // 128
HALO = 16
RC = 8
TM2 = 256
G = 2 * TM2
NG = S // G
_e = lambda k, d: os.environ.get('KCFG_' + k, d)
P1 = [int(v) for v in _e('P1', '256,768,1280').split(',')]
P1SPLIT = int(_e('P1SPLIT', 1280))
SEQ = _e('SEQ', 'AaQqCXxc')
SEQ0 = _e('SEQ0', '')
DEP = int(_e('DEP', 0))
CHAIN = int(_e('CHAIN', 3))
VG = int(_e('VG', 1))
ROT3 = int(_e('ROT3', 0))
BODYONLY = int(_e('BODYONLY', 0))
SCOPES = int(_e('SCOPES', 0))
F32, BF16, U32 = jnp.float32, jnp.bfloat16, jnp.uint32
LOG2E = 1.4426950408889634
QSCALE = DH ** -0.5 * LOG2E

NN = (((1,), (0,)), ((), ()))
NT = (((1,), (1,)), ((), ()))
TN = (((0,), (0,)), ((), ()))

KV_ROWS = []
for _j in range(NT_):
    _h0, _h1 = (128 * _j) // DH, (128 * _j + 127) // DH
    KV_ROWS.append((_h0 * DH // 16 * 16, -(-((_h1 + 1) * DH) // 16) * 16))


def scope(n):
    return jax.named_scope(n) if SCOPES else contextlib.nullcontext()


def _phi(t):
    return jnp.where(t > 0, t + 1.0, jnp.exp(t)) + 1e-6


def _recip(x):
    r = pl.reciprocal(x, approx=True)
    return r * (2.0 - x * r)


def _pack(x):
    return pltpu.bitcast(x.astype(BF16), U32)


def _unpack(x):
    return pltpu.bitcast(x, BF16)


def _zero_after(v):
    b = lax.bitcast_convert_type(v, jnp.int32)
    return jnp.minimum(b & 0x7FFFFFFF, 0)


def _group_sum(a):
    if ROT3:
        return (a + pltpu.roll(a, 64, 1)) + (pltpu.roll(a, 32, 1) + pltpu.roll(a, 96, 1))
    a = a + pltpu.roll(a, 64, 1)
    return a + pltpu.roll(a, 32, 1)


def kernel(xa_hbm, wa_hbm, woa_hbm, xb_hbm, wb_hbm, wob_hbm, out_hbm,
           xa, wa, woa, xb, wb, wob, outv,
           wpT, woap, w2p, tmp, tp, pk0, m_acc, z_acc, zrow, kvs,
           qs0, ks0, vs0, qs1, ks1, vs1, o_s, pqn_s, sems, osems):
    qs, ks, vs = (qs0, qs1), (ks0, ks1), (vs0, vs1)

    def cp(src, dst, k):
        return pltpu.make_async_copy(src, dst, sems.at[k])

    def gather_f32(src, dst):
        for d in range(DH):
            for j in range(NT_):
                dst[d * H // 2:(d + 1) * H // 2, j * 128:(j + 1) * 128] = _pack(src[j, pl.ds(d, H, stride=DH), :])

    def gather_packed(slot, dst, dst_row0):
        for dp in range(DH // 2):
            for j in range(NT_):
                g = tp[slot, j, pl.ds(dp, H, stride=DH // 2), :]
                lo = pltpu.bitcast(g << 16, F32)
                hi = pltpu.bitcast(g & jnp.uint32(0xFFFF0000), F32)
                for e, v in enumerate((lo, hi)):
                    r = (dst_row0 + (2 * dp + e) * H) // 2
                    dst[r:r + H // 2, j * 128:(j + 1) * 128] = _pack(v)

    def perm_T(src, dst_row0, slot):
        for j in range(NT_):
            tp[slot, j] = pltpu.bitcast(src[j * 128:(j + 1) * 128, :].T, U32)
        gather_packed(slot, wpT, dst_row0)

    def perm_rows(src, dst, slot):
        for j in range(NT_):
            tp[slot, j] = pltpu.bitcast(src[:, j * 128:(j + 1) * 128], U32)
        gather_packed(slot, dst, 0)

    def k_proj(r0, r1, c0, c1, nsplit):
        q = (r1 - r0) // nsplit
        return jnp.concatenate(
            [lax.dot_general(xb[r0 + u * q:r0 + (u + 1) * q, :], wb[:, D + c0:D + c1], NN, preferred_element_type=F32)
             for u in range(nsplit)], axis=0)

    def m_update(pk, r0, r1, first):
        zp = pk[0:128]
        for r in range(1, (r1 - r0) // 128):
            zp = zp + pk[r * 128:(r + 1) * 128]
        mm = lax.dot_general(pk.astype(BF16), xb[r0:r1, :], TN, preferred_element_type=F32)
        if first:
            z_acc[...] = zp
            m_acc[...] = mm
        else:
            z_acc[...] += zp
            m_acc[...] += mm

    def B1(r0, r1):
        pk = _phi(jnp.concatenate([k_proj(r0, r1, 0, 512, 1), k_proj(r0, r1, 512, D, 4)], axis=1))
        m_update(pk, r0, r1, False)

    def mid_z():
        tmp[0] = z_acc[...].T
        zt = jnp.concatenate([tmp[0, pl.ds(d, H, stride=DH), :] for d in range(DH)], axis=0)
        zrow[...] = jnp.broadcast_to(jnp.sum(zt.T, axis=0, keepdims=True), (8, D))

    def mid_kv():
        for j in range(NT_):
            r0, r1 = KV_ROWS[j]
            kv = lax.dot_general(m_acc[r0:r1, :].astype(BF16), wb[:, 2 * D + j * 128:2 * D + (j + 1) * 128], NN, preferred_element_type=F32)
            row = lax.broadcasted_iota(jnp.int32, kv.shape, 0) + r0
            col = lax.broadcasted_iota(jnp.int32, kv.shape, 1) + j * 128
            same = (row * 3277 >> 16) == (col * 3277 >> 16)
            kvs[j, 0:(r1 - r0) // 2, :] = _pack(jnp.where(same, kv, 0.0))

    def mid_w2():
        prev_end = 0
        for j in range(NT_):
            r0, r1 = KV_ROWS[j]
            w2 = lax.dot_general(_unpack(kvs[j, 0:(r1 - r0) // 2, :]), wob[j * 128:(j + 1) * 128, :], NN, preferred_element_type=F32)
            ov = prev_end - r0
            for t in range(NT_):
                if ov > 0:
                    tmp[t, r0:prev_end, :] += w2[0:ov, t * 128:(t + 1) * 128]
                tmp[t, prev_end:r1, :] = w2[ov:, t * 128:(t + 1) * 128]
            prev_end = r1
        gather_f32(tmp, w2p)

    def A1(g0, s, first):
        x = xa[pl.ds(g0 + s * TM2, TM2), :]
        res = lax.dot_general(x, _unpack(wpT[0:3 * D // 2, :]), NT, preferred_element_type=F32)
        for t in range(NT_):
            qs[s][t] = res[:, t * 128:(t + 1) * 128] * QSCALE
            for ref, p in ((ks, 1), (vs, 2)):
                if not (first and s == 0):
                    ref[s][t, 0:HALO, :] = ref[1 - s][t, TM2:TM2 + HALO, :]
                ref[s][t, HALO:HALO + TM2, :] = res[:, p * D + t * 128:p * D + (t + 1) * 128]
        return res

    def A2(s, masked, zs, hist):
        pend = None
        for c0 in range(0, TM2, RC):
            if VG:
                z = zs[s][(c0 // RC) % 2]
            else:
                z = zs.pop(0)
            q = [qs[s][t, pl.ds(c0 + z, RC), :] for t in range(NT_)]
            if VG and DEP and len(hist) >= DEP:
                gate = hist[-DEP] < -1.0 if CHAIN == 1 else hist[-DEP] > 3.3e38
                q = [jnp.where(gate, 0.0, x) for x in q]
            ls = []
            for w in range(W):
                o0 = HALO + c0 - DIL * w
                a = q[0] * ks[s][0, pl.ds(o0 + z, RC), :]
                for t in range(1, NT_):
                    a = a + q[t] * ks[s][t, pl.ds(o0 + z, RC), :]
                a = _group_sum(a)
                if masked and c0 < DIL * w:
                    row = lax.broadcasted_iota(jnp.int32, (RC, 128), 0) + c0
                    a = jnp.where(row >= DIL * w, a, -1e30)
                ls.append(a)
            m = functools.reduce(jnp.maximum, ls)
            es = [jnp.exp2(l - m) for l in ls]
            rs = _recip(functools.reduce(jnp.add, es))
            fin = []
            for t in range(NT_):
                o = es[0] * vs[s][t, pl.ds(HALO + c0 + z, RC), :]
                for w in range(1, W):
                    o = o + es[w] * vs[s][t, pl.ds(HALO + c0 - DIL * w + z, RC), :]
                fin.append(o * rs)
            if CHAIN == 3:
                src_v = (fin[0] + fin[1]) + (fin[2] + fin[3]) + fin[4]
            else:
                src_v = {0: m, 1: rs, 2: fin[NT_ - 1]}[CHAIN]
            if VG:
                hist.append(src_v)
            else:
                zs.append(_zero_after(src_v[0, 0]))
            if pend is None:
                pend = fin
            else:
                r = (s * TM2 + c0 - RC) // 2
                for t in range(NT_):
                    o_s[r:r + RC, t * 128:(t + 1) * 128] = _pack(jnp.concatenate([pend[t], fin[t]], axis=0))
                pend = None

    def A3(g0, r, n):
        outv[pl.ds(g0 + r, n), 0:D] = lax.dot_general(
            _unpack(o_s[r // 2:(r + n) // 2, :]), _unpack(woap[...]), NN, preferred_element_type=F32).astype(BF16)

    def B3(g0, s):
        r = s * TM2
        pq = _phi(lax.dot_general(xb[pl.ds(g0 + r, TM2), :], _unpack(wpT[3 * D // 2:4 * D // 2, :]), NT, preferred_element_type=F32))
        z = zrow[0:1, :]
        den = pq[:, 0:128] * z[:, 0:128]
        for t in range(1, NT_):
            den = den + pq[:, t * 128:(t + 1) * 128] * z[:, t * 128:(t + 1) * 128]
        rinv = _recip(_group_sum(den) + 1e-6)
        for t in range(NT_):
            pqn_s[r // 2:(r + TM2) // 2, t * 128:(t + 1) * 128] = _pack(pq[:, t * 128:(t + 1) * 128] * rinv)

    def B4(g0, s):
        r = s * TM2
        outv[pl.ds(g0 + r, TM2), D:2 * D] = lax.dot_general(
            _unpack(pqn_s[r // 2:(r + TM2) // 2, :]), _unpack(w2p[...]), NN, preferred_element_type=F32).astype(BF16)

    def out_copy(row0, n, c0, k):
        return pltpu.make_async_copy(outv.at[pl.ds(row0, n), c0:c0 + D], out_hbm.at[0, pl.ds(row0, n), c0:c0 + D], osems.at[k])

    def out_pieces(seq):
        last = seq[-1]
        res = []
        for ch in seq:
            if ch in 'CcXx':
                r, c0 = (0 if ch in 'CX' else TM2), (0 if ch in 'Cc' else D)
                if ch == last:
                    res += [(ch, r, TM2 // 2, c0), (ch, r + TM2 // 2, TM2 // 2, c0)]
                else:
                    res += [(ch, r, TM2, c0)]
        return res

    def group(g, g0, first, seq):
        pieces = out_pieces(seq)
        zs = {} if VG else []
        hist = []
        for ch in seq:
            s = 0 if ch.isupper() else 1
            if ch in 'Aa':
                res = A1(g0, s, first)
                if VG:
                    zs[s] = [_zero_after(res[TM2 - 1 - i, 3 * D - 1]) for i in range(2)]
                elif ch == 'A':
                    zs.extend(_zero_after(res[TM2 - 1 - i, 3 * D - 1]) for i in range(DEP))
            elif ch in 'Qq':
                B3(g0, s)
            elif ch == 'K':
                mid_kv()
            elif ch == 'W':
                mid_w2()
            else:
                if ch in 'Cc':
                    A2(s, first and s == 0, zs, hist)
                for k, (c2, r, n, c0) in enumerate(pieces):
                    if c2 == ch:
                        if ch in 'Cc':
                            A3(g0, r, n)
                        elif n == TM2:
                            B4(g0, s)
                        else:
                            raise NotImplementedError
                        out_copy(g0 + r, n, c0, g * 5 + k).start()

    def body(g, carry):
        group(g, pl.multiple_of(g * G, G), False, SEQ)
        return carry

    def wait_all():
        for g in range(NG):
            for k, (_, r, n, c0) in enumerate(out_pieces(SEQ0 if (g == 0 and SEQ0 and not BODYONLY) else SEQ)):
                out_copy(g * G + r, n, c0, g * 5 + k).wait()

    if BODYONLY:
        with scope('gl'):
            lax.fori_loop(0, NG, body, 0)
        wait_all()
        return

    cp_x0 = cp(xb_hbm.at[0, 0:256], xb.at[0:256], 0)
    cp_wk0 = cp(wb_hbm.at[:, D:D + 256], wb.at[:, D:D + 256], 1)
    cp_wk1 = cp(wb_hbm.at[:, D + 256:2 * D], wb.at[:, D + 256:2 * D], 2)
    cp_x1 = cp(xb_hbm.at[0, 256:P1SPLIT], xb.at[256:P1SPLIT], 3)
    cp_x2 = cp(xb_hbm.at[0, P1SPLIT:S], xb.at[P1SPLIT:S], 4)
    cp_wa = cp(wa_hbm, wa, 5)
    cp_wq = cp(wb_hbm.at[:, 0:D], wb.at[:, 0:D], 6)
    cp_woa = cp(woa_hbm, woa, 7)
    cp_wv = cp(wb_hbm.at[:, 2 * D:3 * D], wb.at[:, 2 * D:3 * D], 8)
    cp_wob = cp(wob_hbm, wob, 9)
    cp_xa = cp(xa_hbm.at[0], xa, 10)

    with scope('w0'):
        for c in (cp_x0, cp_wk0, cp_wk1, cp_x1, cp_x2, cp_wa, cp_wq, cp_woa, cp_wv, cp_wob, cp_xa):
            c.start()
        for t in range(NT_):
            ks0[t, 0:HALO, :] = jnp.zeros((HALO, 128), F32)
            vs0[t, 0:HALO, :] = jnp.zeros((HALO, 128), F32)
        cp_x0.wait(); cp_wk0.wait()
    with scope('ra'):
        pk0[...] = _phi(k_proj(0, 256, 0, 256, 2))
    with scope('wb'):
        cp_wk1.wait()
    with scope('rb'):
        pk = jnp.concatenate([pk0[...], _phi(k_proj(0, 256, 256, D, 4))], axis=1)
        m_update(pk, 0, 256, True)
    with scope('wc'):
        cp_x1.wait()
    bounds = P1 + [S]
    with scope('rc'):
        for a, b in zip(bounds[:-1], bounds[1:]):
            if a < P1SPLIT:
                B1(a, b)
    with scope('wd'):
        cp_x2.wait(); cp_wa.wait(); cp_wq.wait(); cp_woa.wait()
    with scope('rd'):
        perm_T(wa.at[:, 0:D], 0, 0)
        perm_T(wa.at[:, D:2 * D], D, 1)
        perm_T(wa.at[:, 2 * D:3 * D], 2 * D, 2)
        perm_T(wb.at[:, 0:D], 3 * D, 3)
        perm_rows(woa, woap, 4)
        for a, b in zip(bounds[:-1], bounds[1:]):
            if a >= P1SPLIT:
                B1(a, b)
    with scope('we'):
        cp_wv.wait(); cp_wob.wait(); cp_xa.wait()
    with scope('g0'):
        mid_z()
        group(0, 0, True, SEQ0 or ('K' + SEQ[0] + 'W' + SEQ[1:]))
    with scope('gl'):
        lax.fori_loop(1, NG, body, 0)
    with scope('wf'):
        wait_all()


@jax.jit
def pallas_concat_heads__sliding_local_dilated__linear_attn_block__prompt_kernel(A_x, A_wqkv, A_wo, B_x, B_wqkv, B_wo):
    any_spec = pl.BlockSpec(memory_space=pl.ANY)
    qkv_scratch = [pltpu.VMEM((NT_, TM2, 128), F32), pltpu.VMEM((NT_, TM2 + HALO, 128), F32),
                   pltpu.VMEM((NT_, TM2 + HALO, 128), F32)]
    return pl.pallas_call(
        kernel,
        in_specs=[any_spec] * 6,
        out_specs=any_spec,
        out_shape=jax.ShapeDtypeStruct((1, S, 2 * D), BF16),
        scratch_shapes=[
            pltpu.VMEM((S, D), BF16), pltpu.VMEM((D, 3 * D), BF16), pltpu.VMEM((D, D), BF16),
            pltpu.VMEM((S, D), BF16), pltpu.VMEM((D, 3 * D), BF16), pltpu.VMEM((D, D), BF16),
            pltpu.VMEM((S, 2 * D), BF16),
            pltpu.VMEM((2 * D, D), U32), pltpu.VMEM((D // 2, D), U32), pltpu.VMEM((D // 2, D), U32),
            pltpu.VMEM((NT_, D, 128), F32), pltpu.VMEM((5, NT_, D // 2, 128), U32),
            pltpu.VMEM((256, 256), F32),
            pltpu.VMEM((D, D), F32), pltpu.VMEM((128, D), F32), pltpu.VMEM((8, D), F32),
            pltpu.VMEM((NT_, 80, 128), U32),
            *qkv_scratch, *qkv_scratch,
            pltpu.VMEM((G // 2, D), U32), pltpu.VMEM((G // 2, D), U32),
            pltpu.SemaphoreType.DMA((16,)), pltpu.SemaphoreType.DMA((NG * 5,)),
        ],
        compiler_params=pltpu.CompilerParams(vmem_limit_bytes=100 * 1024 * 1024),
    )(A_x, A_wqkv, A_wo, B_x, B_wqkv, B_wo)
```

```python
import functools

import jax
import jax.numpy as jnp
from jax import lax
import jax.experimental.pallas as pl
import jax.experimental.pallas.tpu as pltpu

S, D, H, DH, W, DIL = 2048, 640, 32, 20, 8, 2
NT_ = D // 128
HALO = 16
RC = 16
TM = 256
G = 2 * TM
NG = S // G
R0, R1 = 640, 1536
KST = (0, 128, 256, 384, 640)
LAST = (0, 192, 256)
SEQ = "AaQqCXxc"
SEQ0 = "AKaWQqCXxc"

F32, BF16, U32 = jnp.float32, jnp.bfloat16, jnp.uint32
LOG2E = 1.4426950408889634
QSCALE = DH ** -0.5 * LOG2E
MASKED = -1e9 * LOG2E

NN = (((1,), (0,)), ((), ()))
NT = (((1,), (1,)), ((), ()))
TN = (((0,), (0,)), ((), ()))

KV_ROWS = ((0, 144, 1), (120, 264, 1), (224, 416, 4), (376, 520, 1), (496, 640, 1))
KV_ORDER = (0, 1, 3, 4, 2)
for _j, (_r0, _r1, _) in enumerate(KV_ROWS):
    assert _r0 <= (128 * _j) // DH * DH and ((128 * _j + 127) // DH + 1) * DH <= _r1


def _dot(a, b, dims=NN):
    return lax.dot_general(a, b, dims, preferred_element_type=F32)


def _rows_dot(lhs, rhs, nsplit):
    q = lhs.shape[0] // nsplit
    return jnp.concatenate([_dot(lhs[u * q:(u + 1) * q], rhs) for u in range(nsplit)], axis=0)


def _sum(xs):
    return functools.reduce(jnp.add, xs)


def _phi(t):
    return jnp.where(t > 0, t + 1.0, jnp.exp(t)) + 1e-6


def _recip(x):
    r = pl.reciprocal(x, approx=True)
    return r * (2.0 - x * r)


def _pack(x):
    return pltpu.bitcast(x.astype(BF16), U32)


def _unpack(x):
    return pltpu.bitcast(x, BF16)


def _zero_after(v):
    b = v.astype(jnp.int32) if v.dtype == U32 else lax.bitcast_convert_type(v, jnp.int32)
    return jnp.minimum(b & 0x7FFFFFFF, 0)


def _group_sum(a):
    return (a + pltpu.roll(a, 64, 1)) + (pltpu.roll(a, 32, 1) + pltpu.roll(a, 96, 1))


def _kernel(xa_hbm, wa_hbm, woa_hbm, xb_hbm, wb_hbm, wob_hbm, out_hbm,
            xa, wa, woa, xb, wb, wob, outv,
            wpT, woap, w2p, tmp, tmpz, zrow, kvs, m_acc, z_acc,
            qs0, ks0, vs0, qs1, ks1, vs1, o_s, pqn_s, sems, *tp):
    qs, ks, vs = (qs0, qs1), (ks0, ks1), (vs0, vs1)
    osem = sems.at[0]

    def prep(m):
        last = []
        for j in range(NT_):
            if m < 4:
                src = wa.at[:, m * D:(m + 1) * D] if m < 3 else wb.at[:, 0:D]
                v = pltpu.bitcast(src[j * 128:(j + 1) * 128, :].T, U32)
            else:
                v = pltpu.roll(pltpu.bitcast(woa[:, j * 128:(j + 1) * 128], U32), 64, 1)
            tp[m * NT_ + j][0:D // 2, :] = v
            last.append(v[D // 2 - 8:D // 2, :])
        z = _zero_after(functools.reduce(jnp.bitwise_or, last)[0, 0])
        dst, row0 = (wpT, m * D) if m < 4 else (woap, 0)
        for j in range(NT_):
            for dp in range(DH // 2):
                g = tp[m * NT_ + j][pl.ds(dp + z, H, stride=DH // 2), :]
                if m == 4:
                    g = pltpu.roll(g, 64, 1)
                lo = pltpu.bitcast(g << 16, F32)
                hi = pltpu.bitcast(g & jnp.uint32(0xFFFF0000), F32)
                for e, v in enumerate((lo, hi)):
                    r = (row0 + (2 * dp + e) * H) // 2
                    dst[r:r + H // 2, j * 128:(j + 1) * 128] = _pack(v)

    def k_proj(r0, r1):
        x = xb[r0:r1, :]
        return jnp.concatenate([_dot(x, wb[:, D:D + 512]), _rows_dot(x, wb[:, D + 512:2 * D], 4)], axis=1)

    def mz_block(k, r0, r1):
        pk = _phi(k)
        zp = _sum([pk[r:r + 128] for r in range(0, r1 - r0, 128)])
        pkb = pk.astype(BF16)
        if (r1 - r0) % 512 == 0:
            return _dot(pkb, xb[r0:r1, :], TN), zp
        pkt = pkb.T
        return jnp.concatenate([_dot(pkt, xb[r0:r1, 0:512]), _rows_dot(pkt, xb[r0:r1, 512:D], 4)], axis=1), zp

    def mid_z(z):
        zt = jnp.concatenate([tmpz[pl.ds(d + z, H, stride=DH), :] for d in range(DH)], axis=0)
        zrow[...] = jnp.broadcast_to(jnp.sum(zt.T, axis=0, keepdims=True), (8, D))

    def mid_kv(m):
        for j in KV_ORDER:
            r0, r1, nsplit = KV_ROWS[j]
            kv = _rows_dot(m[r0:r1].astype(BF16), wb[:, 2 * D + j * 128:2 * D + (j + 1) * 128], nsplit)
            row = lax.broadcasted_iota(jnp.int32, kv.shape, 0) + r0
            col = lax.broadcasted_iota(jnp.int32, kv.shape, 1) + j * 128
            same = (row * 3277 >> 16) == (col * 3277 >> 16)
            kvs[j, 0:(r1 - r0) // 2, :] = _pack(jnp.where(same, kv, 0.0))

    def mid_w2():
        w2s = {}
        for j in KV_ORDER:
            r0, r1, nsplit = KV_ROWS[j]
            w2s[j] = _rows_dot(_unpack(kvs[j, 0:(r1 - r0) // 2, :]), wob[j * 128:(j + 1) * 128, :], nsplit)
        cuts = sorted({r for r0, r1, _ in KV_ROWS for r in (r0, r1)})
        for a, b in zip(cuts[:-1], cuts[1:]):
            v = _sum([w2s[j][a - r0:b - r0] for j, (r0, r1, _) in enumerate(KV_ROWS) if r0 <= a and b <= r1])
            for t in range(NT_):
                tmp[t, a:b, :] = v[:, t * 128:(t + 1) * 128]

    def mid_w2_gather(z):
        for d in range(DH):
            for j in range(NT_):
                w2p[d * H // 2:(d + 1) * H // 2, j * 128:(j + 1) * 128] = _pack(tmp[j, pl.ds(d + z, H, stride=DH), :])

    def qkv_proj(g0, s, first):
        res = _dot(xa[pl.ds(g0 + s * TM, TM), :], _unpack(wpT[0:3 * D // 2, :]), NT)
        for t in range(NT_):
            qs[s][t] = res[:, t * 128:(t + 1) * 128] * QSCALE
            for ref, p in ((ks, 1), (vs, 2)):
                if not (first and s == 0):
                    ref[s][t, 0:HALO, :] = ref[1 - s][t, TM:TM + HALO, :]
                ref[s][t, HALO:HALO + TM, :] = res[:, p * D + t * 128:p * D + (t + 1) * 128]
        return res

    def attention(s, masked, zs):
        for c0 in range(0, TM, RC):
            z = zs[(c0 // RC) % 2]
            q = [qs[s][t, pl.ds(c0 + z, RC), :] for t in range(NT_)]
            ls = []
            for w in range(W):
                o0 = HALO + c0 - DIL * w
                a = _group_sum(_sum([q[t] * ks[s][t, pl.ds(o0 + z, RC), :] for t in range(NT_)]))
                if masked and c0 < DIL * w:
                    row = lax.broadcasted_iota(jnp.int32, (RC, 128), 0) + c0
                    a = jnp.where(row >= DIL * w, a, MASKED)
                ls.append(a)
            m = functools.reduce(jnp.maximum, ls)
            es = [jnp.exp2(l - m) for l in ls]
            rs = _recip(_sum(es))
            r = (s * TM + c0) // 2
            for t in range(NT_):
                o = _sum([es[w] * vs[s][t, pl.ds(HALO + c0 - DIL * w + z, RC), :] for w in range(W)])
                o_s[r:r + RC // 2, t * 128:(t + 1) * 128] = _pack(o * rs)

    def b_query(g0, s):
        r = s * TM
        raw = _dot(xb[pl.ds(g0 + r, TM), :], _unpack(wpT[3 * D // 2:4 * D // 2, :]), NT)
        pq = _phi(raw)
        z = zrow[0:1, :]
        den = _sum([pq[:, t * 128:(t + 1) * 128] * z[:, t * 128:(t + 1) * 128] for t in range(NT_)])
        rinv = _recip(_group_sum(den) + 1e-6)
        for t in range(NT_):
            pqn_s[r // 2:(r + TM) // 2, t * 128:(t + 1) * 128] = _pack(pq[:, t * 128:(t + 1) * 128] * rinv)
        return raw

    def out_proj(g0, r, n, lhs, w, c0):
        raw = _dot(_unpack(lhs[r // 2:(r + n) // 2, :]), _unpack(w[...]))
        outv[pl.ds(g0 + r, n), c0:c0 + D] = raw.astype(BF16)
        pltpu.make_async_copy(outv.at[pl.ds(g0 + r, n), c0:c0 + D],
                              out_hbm.at[0, pl.ds(g0 + r, n), c0:c0 + D], osem).start()
        return raw

    def group(g0, seq, m=None):
        first = m is not None
        zs = {}
        a_pending, w2_pending = None, False
        for n, ch in enumerate(seq):
            s = 0 if ch.isupper() else 1
            res = None
            if ch in "Aa":
                res = qkv_proj(g0, s, first)
                if first and ch == "A":
                    mid_z(_zero_after(res[0, 0]))
            elif ch in "Qq":
                res = b_query(g0, s)
            elif ch == "K":
                mid_kv(m)
            elif ch == "W":
                mid_w2()
                w2_pending = True
            else:
                if ch in "Cc":
                    attention(s, first and s == 0, zs[s])
                lhs, w, c0 = (o_s, woap, 0) if ch in "Cc" else (pqn_s, w2p, D)
                if n == len(seq) - 1:
                    for a, b in zip(LAST[:-1], LAST[1:]):
                        out_proj(g0, s * TM + a, b - a, lhs, w, c0)
                else:
                    res = out_proj(g0, s * TM, TM, lhs, w, c0)
            if res is None:
                continue
            if a_pending is not None:
                zs[a_pending] = [_zero_after(res[8 * i, 0]) for i in range(2)]
                a_pending = None
            if ch in "Aa":
                a_pending = s
            if w2_pending:
                mid_w2_gather(_zero_after(res[0, 0]))
                w2_pending = False

    def first_step():
        nk = len(KST) - 1
        stages = [[(xb_hbm.at[0, 0:R0, a:b], xb.at[0:R0, a:b]), (wb_hbm.at[a:b, D:2 * D], wb.at[a:b, D:2 * D])]
                  for a, b in zip(KST[:-1], KST[1:])]
        stages.append([(xb_hbm.at[0, R0:R1], xb.at[R0:R1]), (woa_hbm, woa)])
        stages.append([(xb_hbm.at[0, R1:S], xb.at[R1:S]), (wa_hbm, wa), (wb_hbm.at[:, 0:D], wb.at[:, 0:D]),
                       (wb_hbm.at[:, 2 * D:3 * D], wb.at[:, 2 * D:3 * D]), (wob_hbm, wob),
                       (xa_hbm.at[0, 0:G], xa.at[0:G])])
        stages.append([(xa_hbm.at[0, G:S], xa.at[G:S])])
        copies = [[pltpu.make_async_copy(src, dst, sems.at[1 + i]) for src, dst in st]
                  for i, st in enumerate(stages)]

        def wait(i):
            for c in copies[i]:
                c.wait()

        for st in copies:
            for c in st:
                c.start()
        for t in range(NT_):
            ks0[t, 0:HALO, :] = jnp.zeros((HALO, 128), F32)
            vs0[t, 0:HALO, :] = jnp.zeros((HALO, 128), F32)

        k = None
        for i, (a, b) in enumerate(zip(KST[:-1], KST[1:])):
            wait(i)
            part = _rows_dot(xb[0:R0, a:b], wb[a:b, D:2 * D], 4 if b - a == 128 else 2)
            k = part if k is None else k + part
        m_acc[...], z_acc[...] = mz_block(k, 0, R0)

        wait(nk)
        prep(4)
        mm, zp = mz_block(k_proj(R0, R1), R0, R1)
        m_acc[...] += mm
        z_acc[...] += zp

        wait(nk + 1)
        for m in range(4):
            prep(m)
        mm, zp = mz_block(k_proj(R1, S), R1, S)
        tmpz[0:D, :] = (z_acc[...] + zp).T
        group(0, SEQ0, m_acc[...] + mm)
        wait(nk + 2)

    step = pl.program_id(0)
    pl.when(step == 0)(first_step)

    @pl.when(step > 0)
    def _():
        group(pl.multiple_of(step * G, G), SEQ)

    @pl.when(step == NG - 1)
    def _():
        pltpu.make_async_copy(outv, out_hbm.at[0], osem).wait()


@jax.jit
def pallas_concat_heads__sliding_local_dilated__linear_attn_block__prompt_kernel(
    A_x: jax.Array,
    A_wqkv: jax.Array,
    A_wo: jax.Array,
    B_x: jax.Array,
    B_wqkv: jax.Array,
    B_wo: jax.Array,
):
    any_spec = pl.BlockSpec(memory_space=pl.ANY)
    qkv_scratch = [pltpu.VMEM((NT_, TM, 128), F32), pltpu.VMEM((NT_, TM + HALO, 128), F32),
                   pltpu.VMEM((NT_, TM + HALO, 128), F32)]
    return pl.pallas_call(
        _kernel,
        grid=(NG,),
        in_specs=[any_spec] * 6,
        out_specs=any_spec,
        out_shape=jax.ShapeDtypeStruct((1, S, 2 * D), BF16),
        scratch_shapes=[
            pltpu.VMEM((S, D), BF16), pltpu.VMEM((D, 3 * D), BF16), pltpu.VMEM((D, D), BF16),
            pltpu.VMEM((S, D), BF16), pltpu.VMEM((D, 3 * D), BF16), pltpu.VMEM((D, D), BF16),
            pltpu.VMEM((S, 2 * D), BF16),
            pltpu.VMEM((2 * D, D), U32), pltpu.VMEM((D // 2, D), U32), pltpu.VMEM((D // 2, D), U32),
            pltpu.VMEM((NT_, D + 24, 128), F32), pltpu.VMEM((D + 24, 128), F32),
            pltpu.VMEM((8, D), F32), pltpu.VMEM((NT_, 96, 128), U32),
            pltpu.VMEM((D, D), F32), pltpu.VMEM((128, D), F32),
            *qkv_scratch, *qkv_scratch,
            pltpu.VMEM((G // 2, D), U32), pltpu.VMEM((G // 2, D), U32),
            pltpu.SemaphoreType.DMA((len(KST) + 3,)),
            *[pltpu.VMEM((D // 2 + 16, 128), U32)] * (5 * NT_),
        ],
        compiler_params=pltpu.CompilerParams(
            dimension_semantics=("arbitrary",), vmem_limit_bytes=100 * 1024 * 1024,
            disable_bounds_checks=True, disable_semaphore_checks=True),
    )(A_x, A_wqkv, A_wo, B_x, B_wqkv, B_wo)
```

```python
import functools

import jax
import jax.numpy as jnp
from jax import lax
import jax.experimental.pallas as pl
import jax.experimental.pallas.tpu as pltpu

S, D, H, DH, W, DIL = 2048, 640, 32, 20, 8, 2
NT_ = D // 128
HALO = 16
RC = 16
TM = 256
G = 2 * TM
NG = S // G
R0, R1 = 640, 1536
KST = (0, 128, 256, 384, 640)
LAST = (0, 192, 256)
SEQ = "AaQqCXxc"
SEQ0 = "AaKWQqCXxc"

F32, BF16, U32 = jnp.float32, jnp.bfloat16, jnp.uint32
LOG2E = 1.4426950408889634
QSCALE = DH ** -0.5 * LOG2E
MASKED = -1e9 * LOG2E

NN = (((1,), (0,)), ((), ()))
NT = (((1,), (1,)), ((), ()))
TN = (((0,), (0,)), ((), ()))

KV_ROWS = ((0, 144, 1), (120, 264, 1), (224, 416, 4), (376, 520, 1), (496, 640, 1))
KV_ORDER = (0, 1, 3, 4, 2)
for _j, (_r0, _r1, _) in enumerate(KV_ROWS):
    assert _r0 <= (128 * _j) // DH * DH and ((128 * _j + 127) // DH + 1) * DH <= _r1


def _dot(a, b, dims=NN):
    return lax.dot_general(a, b, dims, preferred_element_type=F32)


def _rows_dot(lhs, rhs, nsplit):
    q = lhs.shape[0] // nsplit
    return jnp.concatenate([_dot(lhs[u * q:(u + 1) * q], rhs) for u in range(nsplit)], axis=0)


def _sum(xs):
    return functools.reduce(jnp.add, xs)


def _phi(t):
    return jnp.where(t > 0, t + 1.0, jnp.exp(t)) + 1e-6


def _recip(x):
    r = pl.reciprocal(x, approx=True)
    return r * (2.0 - x * r)


def _pack(x):
    return pltpu.bitcast(x.astype(BF16), U32)


def _unpack(x):
    return pltpu.bitcast(x, BF16)


def _zero_after(v):
    b = v.astype(jnp.int32) if v.dtype == U32 else lax.bitcast_convert_type(v, jnp.int32)
    return jnp.minimum(b & 0x7FFFFFFF, 0)


def _rows(ref, start, z, size, stride=1):
    return pl.ds(jnp.clip(start + z, 0, ref.shape[-2] - size * stride), size, stride=stride)


def _group_sum(a):
    return (a + pltpu.roll(a, 64, 1)) + (pltpu.roll(a, 32, 1) + pltpu.roll(a, 96, 1))


def _kernel(xa_hbm, wa_hbm, woa_hbm, xb_hbm, wb_hbm, wob_hbm, out_hbm,
            xa, wa, woa, xb, wb, wob, outv,
            wpT, woap, w2p, tmp, tmpz, zrow, kvs, m_acc, z_acc,
            qs0, ks0, vs0, qs1, ks1, vs1, o_s, pqn_s, sems, *tp):
    qs, ks, vs = (qs0, qs1), (ks0, ks1), (vs0, vs1)
    osem = sems.at[0]

    def prep(m):
        last = []
        for j in range(NT_):
            if m < 4:
                src = wa.at[:, m * D:(m + 1) * D] if m < 3 else wb.at[:, 0:D]
                v = pltpu.bitcast(src[j * 128:(j + 1) * 128, :].T, U32)
            else:
                v = pltpu.roll(pltpu.bitcast(woa[:, j * 128:(j + 1) * 128], U32), 64, 1)
            tp[m * NT_ + j][0:D // 2, :] = v
            last.append(v[D // 2 - 8:D // 2, :])
        z = _zero_after(functools.reduce(jnp.bitwise_or, last)[0, 0])
        sl = [_rows(tp[0], dp, z, H, DH // 2) for dp in range(DH // 2)]
        dst, row0 = (wpT, m * D) if m < 4 else (woap, 0)
        for j in range(NT_):
            for dp in range(DH // 2):
                g = tp[m * NT_ + j][sl[dp], :]
                if m == 4:
                    g = pltpu.roll(g, 64, 1)
                lo = pltpu.bitcast(g << 16, F32)
                hi = pltpu.bitcast(g & jnp.uint32(0xFFFF0000), F32)
                for e, v in enumerate((lo, hi)):
                    r = (row0 + (2 * dp + e) * H) // 2
                    dst[r:r + H // 2, j * 128:(j + 1) * 128] = _pack(v)

    def k_proj(r0, r1):
        x = xb[r0:r1, :]
        return jnp.concatenate([_dot(x, wb[:, D:D + 512]), _rows_dot(x, wb[:, D + 512:2 * D], 4)], axis=1)

    def mz_block(k, r0, r1):
        pk = _phi(k)
        zp = _sum([pk[r:r + 128] for r in range(0, r1 - r0, 128)])
        pkb = pk.astype(BF16)
        if (r1 - r0) % 512 == 0:
            return _dot(pkb, xb[r0:r1, :], TN), zp
        pkt = pkb.T
        return jnp.concatenate([_dot(pkt, xb[r0:r1, 0:512]), _rows_dot(pkt, xb[r0:r1, 512:D], 4)], axis=1), zp

    def mid_z(z):
        zt = jnp.concatenate([tmpz[_rows(tmpz, d, z, H, DH), :] for d in range(DH)], axis=0)
        zrow[...] = jnp.broadcast_to(jnp.sum(zt.T, axis=0, keepdims=True), (8, D))

    def mid_kv(m):
        for j in KV_ORDER:
            r0, r1, nsplit = KV_ROWS[j]
            kv = _rows_dot(m[r0:r1].astype(BF16), wb[:, 2 * D + j * 128:2 * D + (j + 1) * 128], nsplit)
            row = lax.broadcasted_iota(jnp.int32, kv.shape, 0) + r0
            col = lax.broadcasted_iota(jnp.int32, kv.shape, 1) + j * 128
            same = (row * 3277 >> 16) == (col * 3277 >> 16)
            kvs[j, 0:(r1 - r0) // 2, :] = _pack(jnp.where(same, kv, 0.0))

    def mid_w2():
        w2s = {}
        for j in KV_ORDER:
            r0, r1, nsplit = KV_ROWS[j]
            w2s[j] = _rows_dot(_unpack(kvs[j, 0:(r1 - r0) // 2, :]), wob[j * 128:(j + 1) * 128, :], nsplit)
        cuts = sorted({r for r0, r1, _ in KV_ROWS for r in (r0, r1)})
        for a, b in zip(cuts[:-1], cuts[1:]):
            v = _sum([w2s[j][a - r0:b - r0] for j, (r0, r1, _) in enumerate(KV_ROWS) if r0 <= a and b <= r1])
            for t in range(NT_):
                tmp[t, a:b, :] = v[:, t * 128:(t + 1) * 128]

    def mid_w2_gather(z):
        for d in range(DH):
            sl = _rows(tmp, d, z, H, DH)
            for j in range(NT_):
                w2p[d * H // 2:(d + 1) * H // 2, j * 128:(j + 1) * 128] = _pack(tmp[j, sl, :])

    def qkv_proj(g0, s, first):
        res = _dot(xa[pl.ds(g0 + s * TM, TM), :], _unpack(wpT[0:3 * D // 2, :]), NT)
        for t in range(NT_):
            qs[s][t] = res[:, t * 128:(t + 1) * 128] * QSCALE
            for ref, p in ((ks, 1), (vs, 2)):
                if not (first and s == 0):
                    ref[s][t, 0:HALO, :] = ref[1 - s][t, TM:TM + HALO, :]
                ref[s][t, HALO:HALO + TM, :] = res[:, p * D + t * 128:p * D + (t + 1) * 128]
        return res

    def attention(s, masked, zs):
        for c0 in range(0, TM, RC):
            z = zs[(c0 // RC) % 2]
            sl = [_rows(ks0, HALO + c0 - DIL * w, z, RC) for w in range(W)]
            slq = _rows(qs0, c0, z, RC)
            q = [qs[s][t, slq, :] for t in range(NT_)]
            ls = []
            for w in range(W):
                a = _group_sum(_sum([q[t] * ks[s][t, sl[w], :] for t in range(NT_)]))
                if masked and c0 < DIL * w:
                    row = lax.broadcasted_iota(jnp.int32, (RC, 128), 0) + c0
                    a = jnp.where(row >= DIL * w, a, MASKED)
                ls.append(a)
            m = functools.reduce(jnp.maximum, ls)
            es = [jnp.exp2(l - m) for l in ls]
            rs = _recip(_sum(es))
            r = (s * TM + c0) // 2
            for t in range(NT_):
                o = _sum([es[w] * vs[s][t, sl[w], :] for w in range(W)])
                o_s[r:r + RC // 2, t * 128:(t + 1) * 128] = _pack(o * rs)

    def b_query(g0, s):
        r = s * TM
        raw = _dot(xb[pl.ds(g0 + r, TM), :], _unpack(wpT[3 * D // 2:4 * D // 2, :]), NT)
        pq = _phi(raw)
        z = zrow[0:1, :]
        den = _sum([pq[:, t * 128:(t + 1) * 128] * z[:, t * 128:(t + 1) * 128] for t in range(NT_)])
        rinv = _recip(_group_sum(den) + 1e-6)
        for t in range(NT_):
            pqn_s[r // 2:(r + TM) // 2, t * 128:(t + 1) * 128] = _pack(pq[:, t * 128:(t + 1) * 128] * rinv)
        return raw

    def out_proj(g0, r, n, lhs, w, c0):
        raw = _dot(_unpack(lhs[r // 2:(r + n) // 2, :]), _unpack(w[...]))
        outv[pl.ds(g0 + r, n), c0:c0 + D] = raw.astype(BF16)
        pltpu.make_async_copy(outv.at[pl.ds(g0 + r, n), c0:c0 + D],
                              out_hbm.at[0, pl.ds(g0 + r, n), c0:c0 + D], osem).start()
        return raw

    def group(g0, seq, m=None):
        first = m is not None
        zs = {}
        a_pending, w2_pending = None, False
        for n, ch in enumerate(seq):
            s = 0 if ch.isupper() else 1
            res = None
            if ch in "Aa":
                res = qkv_proj(g0, s, first)
                if first and ch == "A":
                    mid_z(_zero_after(res[0, 0]))
            elif ch in "Qq":
                res = b_query(g0, s)
            elif ch == "K":
                mid_kv(m)
            elif ch == "W":
                mid_w2()
                w2_pending = True
            else:
                if ch in "Cc":
                    attention(s, first and s == 0, zs[s])
                lhs, w, c0 = (o_s, woap, 0) if ch in "Cc" else (pqn_s, w2p, D)
                if n == len(seq) - 1:
                    for a, b in zip(LAST[:-1], LAST[1:]):
                        out_proj(g0, s * TM + a, b - a, lhs, w, c0)
                else:
                    res = out_proj(g0, s * TM, TM, lhs, w, c0)
            if res is None:
                continue
            if a_pending is not None:
                zs[a_pending] = [_zero_after(res[8 * i, 128]) for i in range(2)]
                a_pending = None
            if ch in "Aa":
                a_pending = s
            if w2_pending:
                mid_w2_gather(_zero_after(res[0, 128]))
                w2_pending = False

    def first_step():
        nk = len(KST) - 1
        stages = [[(xb_hbm.at[0, 0:R0, a:b], xb.at[0:R0, a:b]), (wb_hbm.at[a:b, D:2 * D], wb.at[a:b, D:2 * D])]
                  for a, b in zip(KST[:-1], KST[1:])]
        stages.append([(xb_hbm.at[0, R0:R1], xb.at[R0:R1]), (woa_hbm, woa)])
        stages.append([(xb_hbm.at[0, R1:S], xb.at[R1:S]), (wa_hbm, wa), (wb_hbm.at[:, 0:D], wb.at[:, 0:D]),
                       (wb_hbm.at[:, 2 * D:3 * D], wb.at[:, 2 * D:3 * D]), (wob_hbm, wob),
                       (xa_hbm.at[0, 0:G], xa.at[0:G])])
        stages.append([(xa_hbm.at[0, G:S], xa.at[G:S])])
        copies = [[pltpu.make_async_copy(src, dst, sems.at[1 + i]) for src, dst in st]
                  for i, st in enumerate(stages)]

        def wait(i):
            for c in copies[i]:
                c.wait()

        for st in copies:
            for c in st:
                c.start()
        for t in range(NT_):
            ks0[t, 0:HALO, :] = jnp.zeros((HALO, 128), F32)
            vs0[t, 0:HALO, :] = jnp.zeros((HALO, 128), F32)
            tmp[t, D:D + 24, :] = jnp.zeros((24, 128), F32)
        tmpz[D:D + 24, :] = jnp.zeros((24, 128), F32)
        for ref in tp:
            ref[D // 2:D // 2 + 16, :] = jnp.zeros((16, 128), U32)

        k = None
        for i, (a, b) in enumerate(zip(KST[:-1], KST[1:])):
            wait(i)
            part = _rows_dot(xb[0:R0, a:b], wb[a:b, D:2 * D], 4 if b - a == 128 else 2)
            k = part if k is None else k + part
        m_acc[...], z_acc[...] = mz_block(k, 0, R0)

        wait(nk)
        prep(4)
        mm, zp = mz_block(k_proj(R0, R1), R0, R1)
        m_acc[...] += mm
        z_acc[...] += zp

        wait(nk + 1)
        for m in range(4):
            prep(m)
        mm, zp = mz_block(k_proj(R1, S), R1, S)
        tmpz[0:D, :] = (z_acc[...] + zp).T
        group(0, SEQ0, m_acc[...] + mm)
        wait(nk + 2)

    step = pl.program_id(0)
    pl.when(step == 0)(first_step)

    @pl.when(step > 0)
    def _():
        group(pl.multiple_of(step * G, G), SEQ)

    @pl.when(step == NG - 1)
    def _():
        pltpu.make_async_copy(outv, out_hbm.at[0], osem).wait()


@jax.jit
def pallas_concat_heads__sliding_local_dilated__linear_attn_block__prompt_kernel(
    A_x: jax.Array,
    A_wqkv: jax.Array,
    A_wo: jax.Array,
    B_x: jax.Array,
    B_wqkv: jax.Array,
    B_wo: jax.Array,
):
    any_spec = pl.BlockSpec(memory_space=pl.ANY)
    qkv_scratch = [pltpu.VMEM((NT_, TM, 128), F32), pltpu.VMEM((NT_, TM + HALO, 128), F32),
                   pltpu.VMEM((NT_, TM + HALO, 128), F32)]
    return pl.pallas_call(
        _kernel,
        grid=(NG,),
        in_specs=[any_spec] * 6,
        out_specs=any_spec,
        out_shape=jax.ShapeDtypeStruct((1, S, 2 * D), BF16),
        scratch_shapes=[
            pltpu.VMEM((S, D), BF16), pltpu.VMEM((D, 3 * D), BF16), pltpu.VMEM((D, D), BF16),
            pltpu.VMEM((S, D), BF16), pltpu.VMEM((D, 3 * D), BF16), pltpu.VMEM((D, D), BF16),
            pltpu.VMEM((S, 2 * D), BF16),
            pltpu.VMEM((2 * D, D), U32), pltpu.VMEM((D // 2, D), U32), pltpu.VMEM((D // 2, D), U32),
            pltpu.VMEM((NT_, D + 24, 128), F32), pltpu.VMEM((D + 24, 128), F32),
            pltpu.VMEM((8, D), F32), pltpu.VMEM((NT_, 96, 128), U32),
            pltpu.VMEM((D, D), F32), pltpu.VMEM((128, D), F32),
            *qkv_scratch, *qkv_scratch,
            pltpu.VMEM((G // 2, D), U32), pltpu.VMEM((G // 2, D), U32),
            pltpu.SemaphoreType.DMA((len(KST) + 3,)),
            *[pltpu.VMEM((D // 2 + 16, 128), U32)] * (5 * NT_),
        ],
        compiler_params=pltpu.CompilerParams(
            dimension_semantics=("arbitrary",), vmem_limit_bytes=100 * 1024 * 1024,
            disable_bounds_checks=True, disable_semaphore_checks=True),
    )(A_x, A_wqkv, A_wo, B_x, B_wqkv, B_wo)
```

```python
import functools

import jax
import jax.numpy as jnp
from jax import lax
import jax.experimental.pallas as pl
import jax.experimental.pallas.tpu as pltpu

S, D, H, DH, W, DIL = 2048, 640, 32, 20, 8, 2
NT_ = D // 128
HALO = 16
RC = 16
TM = 256
G = 2 * TM
NG = S // G
R0, R1 = 640, 1536
KST = (0, 128, 256, 384, 640)
LAST = (0, 192, 256)
SEQ = "AaQqCXxc"
SEQ0 = "AaKWQqCXxc"

F32, BF16, U32 = jnp.float32, jnp.bfloat16, jnp.uint32
LOG2E = 1.4426950408889634
QSCALE = DH ** -0.5 * LOG2E
MASKED = -1e9 * LOG2E

NN = (((1,), (0,)), ((), ()))
NT = (((1,), (1,)), ((), ()))
TN = (((0,), (0,)), ((), ()))

KV_ROWS = ((0, 144, 1), (120, 264, 1), (240, 400, (32, 32, 48, 48)), (376, 520, 1), (496, 640, 1))
KV_ORDER = (0, 1, 3, 4, 2)
for _j, (_r0, _r1, _) in enumerate(KV_ROWS):
    assert _r0 <= (128 * _j) // DH * DH and ((128 * _j + 127) // DH + 1) * DH <= _r1


def _dot(a, b, dims=NN):
    return lax.dot_general(a, b, dims, preferred_element_type=F32)


def _rows_dot(lhs, rhs, split):
    sizes = (lhs.shape[0] // split,) * split if isinstance(split, int) else split
    starts = [sum(sizes[:u]) for u in range(len(sizes))]
    return jnp.concatenate([_dot(lhs[a:a + n], rhs) for a, n in zip(starts, sizes)], axis=0)


def _sum(xs):
    return functools.reduce(jnp.add, xs)


def _phi(t):
    return jnp.where(t > 0, t + 1.0, jnp.exp(t)) + 1e-6


def _recip(x):
    r = pl.reciprocal(x, approx=True)
    return r * (2.0 - x * r)


def _pack(x):
    return pltpu.bitcast(x.astype(BF16), U32)


def _unpack(x):
    return pltpu.bitcast(x, BF16)


def _zero_after(v):
    b = v.astype(jnp.int32) if v.dtype == U32 else lax.bitcast_convert_type(v, jnp.int32)
    return jnp.minimum(b & 0x7FFFFFFF, 0)


def _rows(ref, start, z, size, stride=1):
    return pl.ds(jnp.clip(start + z, 0, ref.shape[-2] - size * stride), size, stride=stride)


def _group_sum(a):
    return (a + pltpu.roll(a, 64, 1)) + (pltpu.roll(a, 32, 1) + pltpu.roll(a, 96, 1))


def _kernel(xa_hbm, wa_hbm, woa_hbm, xb_hbm, wb_hbm, wob_hbm, out_hbm,
            xa, wa, woa, xb, wb, wob, outv,
            wpT, woap, w2p, tmp, tmpz, zrow, kvs, m_acc, z_acc,
            qs0, ks0, vs0, qs1, ks1, vs1, o_s, pqn_s, sems, *tp):
    qs, ks, vs = (qs0, qs1), (ks0, ks1), (vs0, vs1)
    osem = sems.at[0]

    def prep(m):
        last = []
        for j in range(NT_):
            if m < 4:
                src = wa.at[:, m * D:(m + 1) * D] if m < 3 else wb.at[:, 0:D]
                v = pltpu.bitcast(src[j * 128:(j + 1) * 128, :].T, U32)
            else:
                v = pltpu.roll(pltpu.bitcast(woa[:, j * 128:(j + 1) * 128], U32), 64, 1)
            tp[m * NT_ + j][0:D // 2, :] = v
            last.append(v[D // 2 - 8:D // 2, :])
        z = _zero_after(functools.reduce(jnp.bitwise_or, last)[0, 0])
        sl = [_rows(tp[0], dp, z, H, DH // 2) for dp in range(DH // 2)]
        dst, row0 = (wpT, m * D) if m < 4 else (woap, 0)
        for j in range(NT_):
            for dp in range(DH // 2):
                g = tp[m * NT_ + j][sl[dp], :]
                if m == 4:
                    g = pltpu.roll(g, 64, 1)
                lo = pltpu.bitcast(g << 16, F32)
                hi = pltpu.bitcast(g & jnp.uint32(0xFFFF0000), F32)
                for e, v in enumerate((lo, hi)):
                    r = (row0 + (2 * dp + e) * H) // 2
                    dst[r:r + H // 2, j * 128:(j + 1) * 128] = _pack(v)

    def k_proj(r0, r1):
        x = xb[r0:r1, :]
        return jnp.concatenate([_dot(x, wb[:, D:D + 512]), _rows_dot(x, wb[:, D + 512:2 * D], 4)], axis=1)

    def mz_block(k, r0, r1):
        pk = _phi(k)
        zp = _sum([pk[r:r + 128] for r in range(0, r1 - r0, 128)])
        pkb = pk.astype(BF16)
        if (r1 - r0) % 512 == 0:
            return _dot(pkb, xb[r0:r1, :], TN), zp
        pkt = pkb.T
        return jnp.concatenate([_dot(pkt, xb[r0:r1, 0:512]), _rows_dot(pkt, xb[r0:r1, 512:D], 4)], axis=1), zp

    def mid_z(z):
        zt = jnp.concatenate([tmpz[_rows(tmpz, d, z, H, DH), :] for d in range(DH)], axis=0)
        zrow[...] = jnp.broadcast_to(jnp.sum(zt.T, axis=0, keepdims=True), (8, D))

    def mid_kv(m):
        for j in KV_ORDER:
            r0, r1, split = KV_ROWS[j]
            kv = _rows_dot(m[r0:r1].astype(BF16), wb[:, 2 * D + j * 128:2 * D + (j + 1) * 128], split)
            row = lax.broadcasted_iota(jnp.int32, kv.shape, 0) + r0
            col = lax.broadcasted_iota(jnp.int32, kv.shape, 1) + j * 128
            same = (row * 3277 >> 16) == (col * 3277 >> 16)
            kvs[j, 0:(r1 - r0) // 2, :] = _pack(jnp.where(same, kv, 0.0))

    def mid_w2():
        w2s = {}
        for j in KV_ORDER:
            r0, r1, split = KV_ROWS[j]
            w2s[j] = _rows_dot(_unpack(kvs[j, 0:(r1 - r0) // 2, :]), wob[j * 128:(j + 1) * 128, :], split)
        cuts = sorted({r for r0, r1, _ in KV_ROWS for r in (r0, r1)})
        for a, b in zip(cuts[:-1], cuts[1:]):
            v = _sum([w2s[j][a - r0:b - r0] for j, (r0, r1, _) in enumerate(KV_ROWS) if r0 <= a and b <= r1])
            for t in range(NT_):
                tmp[t, a:b, :] = v[:, t * 128:(t + 1) * 128]

    def mid_w2_gather(z):
        for d in range(DH):
            sl = _rows(tmp, d, z, H, DH)
            for j in range(NT_):
                w2p[d * H // 2:(d + 1) * H // 2, j * 128:(j + 1) * 128] = _pack(tmp[j, sl, :])

    def qkv_proj(g0, s, first):
        res = _dot(xa[pl.ds(g0 + s * TM, TM), :], _unpack(wpT[0:3 * D // 2, :]), NT)
        for t in range(NT_):
            qs[s][t] = res[:, t * 128:(t + 1) * 128] * QSCALE
            for ref, p in ((ks, 1), (vs, 2)):
                if not (first and s == 0):
                    ref[s][t, 0:HALO, :] = ref[1 - s][t, TM:TM + HALO, :]
                ref[s][t, HALO:HALO + TM, :] = res[:, p * D + t * 128:p * D + (t + 1) * 128]
        return res

    def attention(s, masked, zs):
        for c0 in range(0, TM, RC):
            z = zs[(c0 // RC) % 2]
            sl = [_rows(ks0, HALO + c0 - DIL * w, z, RC) for w in range(W)]
            slq = _rows(qs0, c0, z, RC)
            q = [qs[s][t, slq, :] for t in range(NT_)]
            ls = []
            for w in range(W):
                a = _group_sum(_sum([q[t] * ks[s][t, sl[w], :] for t in range(NT_)]))
                if masked and c0 < DIL * w:
                    row = lax.broadcasted_iota(jnp.int32, (RC, 128), 0) + c0
                    a = jnp.where(row >= DIL * w, a, MASKED)
                ls.append(a)
            m = functools.reduce(jnp.maximum, ls)
            es = [jnp.exp2(l - m) for l in ls]
            rs = _recip(_sum(es))
            r = (s * TM + c0) // 2
            for t in range(NT_):
                o = _sum([es[w] * vs[s][t, sl[w], :] for w in range(W)])
                o_s[r:r + RC // 2, t * 128:(t + 1) * 128] = _pack(o * rs)

    def b_query(g0, s):
        r = s * TM
        raw = _dot(xb[pl.ds(g0 + r, TM), :], _unpack(wpT[3 * D // 2:4 * D // 2, :]), NT)
        pq = _phi(raw)
        z = zrow[0:1, :]
        den = _sum([pq[:, t * 128:(t + 1) * 128] * z[:, t * 128:(t + 1) * 128] for t in range(NT_)])
        rinv = _recip(_group_sum(den) + 1e-6)
        for t in range(NT_):
            pqn_s[r // 2:(r + TM) // 2, t * 128:(t + 1) * 128] = _pack(pq[:, t * 128:(t + 1) * 128] * rinv)
        return raw

    def out_proj(g0, r, n, lhs, w, c0):
        raw = _dot(_unpack(lhs[r // 2:(r + n) // 2, :]), _unpack(w[...]))
        outv[pl.ds(g0 + r, n), c0:c0 + D] = raw.astype(BF16)
        pltpu.make_async_copy(outv.at[pl.ds(g0 + r, n), c0:c0 + D],
                              out_hbm.at[0, pl.ds(g0 + r, n), c0:c0 + D], osem).start()
        return raw

    def group(g0, seq, m=None):
        first = m is not None
        zs = {}
        a_pending, w2_pending = None, False
        for n, ch in enumerate(seq):
            s = 0 if ch.isupper() else 1
            res = None
            if ch in "Aa":
                res = qkv_proj(g0, s, first)
                if first and ch == "A":
                    mid_z(_zero_after(res[0, 0]))
            elif ch in "Qq":
                res = b_query(g0, s)
            elif ch == "K":
                mid_kv(m)
            elif ch == "W":
                mid_w2()
                w2_pending = True
            else:
                if ch in "Cc":
                    attention(s, first and s == 0, zs[s])
                lhs, w, c0 = (o_s, woap, 0) if ch in "Cc" else (pqn_s, w2p, D)
                if n == len(seq) - 1:
                    for a, b in zip(LAST[:-1], LAST[1:]):
                        out_proj(g0, s * TM + a, b - a, lhs, w, c0)
                else:
                    res = out_proj(g0, s * TM, TM, lhs, w, c0)
            if res is None:
                continue
            if a_pending is not None:
                zs[a_pending] = [_zero_after(res[8 * i, 128]) for i in range(2)]
                a_pending = None
            if ch in "Aa":
                a_pending = s
            if w2_pending:
                mid_w2_gather(_zero_after(res[0, 128]))
                w2_pending = False

    def first_step():
        nk = len(KST) - 1
        stages = [[(xb_hbm.at[0, 0:R0, a:b], xb.at[0:R0, a:b]), (wb_hbm.at[a:b, D:2 * D], wb.at[a:b, D:2 * D])]
                  for a, b in zip(KST[:-1], KST[1:])]
        stages.append([(xb_hbm.at[0, R0:R1], xb.at[R0:R1]), (woa_hbm, woa)])
        stages.append([(xb_hbm.at[0, R1:S], xb.at[R1:S]), (wa_hbm, wa), (wb_hbm.at[:, 0:D], wb.at[:, 0:D]),
                       (wb_hbm.at[:, 2 * D:3 * D], wb.at[:, 2 * D:3 * D]), (wob_hbm, wob),
                       (xa_hbm.at[0, 0:G], xa.at[0:G])])
        stages.append([(xa_hbm.at[0, G:S], xa.at[G:S])])
        copies = [[pltpu.make_async_copy(src, dst, sems.at[1 + i]) for src, dst in st]
                  for i, st in enumerate(stages)]

        def wait(i):
            for c in copies[i]:
                c.wait()

        for st in copies:
            for c in st:
                c.start()
        for t in range(NT_):
            ks0[t, 0:HALO, :] = jnp.zeros((HALO, 128), F32)
            vs0[t, 0:HALO, :] = jnp.zeros((HALO, 128), F32)
            tmp[t, D:D + 24, :] = jnp.zeros((24, 128), F32)
        tmpz[D:D + 24, :] = jnp.zeros((24, 128), F32)
        for ref in tp:
            ref[D // 2:D // 2 + 16, :] = jnp.zeros((16, 128), U32)

        k = None
        for i, (a, b) in enumerate(zip(KST[:-1], KST[1:])):
            wait(i)
            part = _rows_dot(xb[0:R0, a:b], wb[a:b, D:2 * D], 4 if b - a == 128 else 2)
            k = part if k is None else k + part
        m_acc[...], z_acc[...] = mz_block(k, 0, R0)

        wait(nk)
        prep(4)
        mm, zp = mz_block(k_proj(R0, R1), R0, R1)
        m_acc[...] += mm
        z_acc[...] += zp

        wait(nk + 1)
        for m in range(4):
            prep(m)
        mm, zp = mz_block(k_proj(R1, S), R1, S)
        tmpz[0:D, :] = (z_acc[...] + zp).T
        group(0, SEQ0, m_acc[...] + mm)
        wait(nk + 2)

    step = pl.program_id(0)
    pl.when(step == 0)(first_step)

    @pl.when(step > 0)
    def _():
        group(pl.multiple_of(step * G, G), SEQ)

    @pl.when(step == NG - 1)
    def _():
        pltpu.make_async_copy(outv, out_hbm.at[0], osem).wait()


@jax.jit
def pallas_concat_heads__sliding_local_dilated__linear_attn_block__prompt_kernel(
    A_x: jax.Array,
    A_wqkv: jax.Array,
    A_wo: jax.Array,
    B_x: jax.Array,
    B_wqkv: jax.Array,
    B_wo: jax.Array,
):
    any_spec = pl.BlockSpec(memory_space=pl.ANY)
    qkv_scratch = [pltpu.VMEM((NT_, TM, 128), F32), pltpu.VMEM((NT_, TM + HALO, 128), F32),
                   pltpu.VMEM((NT_, TM + HALO, 128), F32)]
    return pl.pallas_call(
        _kernel,
        grid=(NG,),
        in_specs=[any_spec] * 6,
        out_specs=any_spec,
        out_shape=jax.ShapeDtypeStruct((1, S, 2 * D), BF16),
        scratch_shapes=[
            pltpu.VMEM((S, D), BF16), pltpu.VMEM((D, 3 * D), BF16), pltpu.VMEM((D, D), BF16),
            pltpu.VMEM((S, D), BF16), pltpu.VMEM((D, 3 * D), BF16), pltpu.VMEM((D, D), BF16),
            pltpu.VMEM((S, 2 * D), BF16),
            pltpu.VMEM((2 * D, D), U32), pltpu.VMEM((D // 2, D), U32), pltpu.VMEM((D // 2, D), U32),
            pltpu.VMEM((NT_, D + 24, 128), F32), pltpu.VMEM((D + 24, 128), F32),
            pltpu.VMEM((8, D), F32), pltpu.VMEM((NT_, 80, 128), U32),
            pltpu.VMEM((D, D), F32), pltpu.VMEM((128, D), F32),
            *qkv_scratch, *qkv_scratch,
            pltpu.VMEM((G // 2, D), U32), pltpu.VMEM((G // 2, D), U32),
            pltpu.SemaphoreType.DMA((len(KST) + 3,)),
            *[pltpu.VMEM((D // 2 + 16, 128), U32)] * (5 * NT_),
        ],
        compiler_params=pltpu.CompilerParams(
            dimension_semantics=("arbitrary",), vmem_limit_bytes=100 * 1024 * 1024,
            disable_bounds_checks=True, disable_semaphore_checks=True),
    )(A_x, A_wqkv, A_wo, B_x, B_wqkv, B_wo)
```
